```python
import jax
import jax.numpy as jnp

def _softmax(x, axis=-1):
    return jax.nn.softmax(x, axis=axis)

def _gelu(x):
    return jax.nn.gelu(x, approximate=True)

def _silu(x):
    return jax.nn.silu(x)

def _sigmoid(x):
    return jax.nn.sigmoid(x)

def _layernorm(x, axis=-1, eps=1e-05):
    m = jnp.mean(x, axis=axis, keepdims=True)
    v = jnp.var(x, axis=axis, keepdims=True)
    return (x - m) / jnp.sqrt(v + eps)

def _scatter_add(tgt, idx, src, axis=0):
    return tgt.at[idx].add(src)

def _segment_sum(src, seg, n):
    return jax.ops.segment_sum(src, seg, n)

class _Rng:

    def __init__(self, key):
        self._k = key

    def _next(self):
        self._k, sub = jax.random.split(self._k)
        return sub

    def normal(self, shape):
        return jax.random.normal(self._next(), shape, dtype=jnp.bfloat16)

    def randint(self, lo, hi, shape):
        return jax.random.randint(self._next(), shape, lo, hi, dtype=jnp.int32)

    def uniform(self, shape, lo=0.0, hi=1.0):
        return jax.random.uniform(self._next(), shape, jnp.bfloat16, lo, hi)

    def permutation(self, n):
        return jax.random.permutation(self._next(), n)
kernel_name = 'concat_heads__compressed_kv_cla__memory_aug_recurrent_mem_tr__prompt'

def setup_inputs():
    _rng = _Rng(jax.random.key(int.from_bytes(__import__("os").urandom(4), "little")))
    _w = lambda a: (lambda t: t.astype(jnp.bfloat16) if jnp.issubdtype(t.dtype, jnp.floating) else t)(jnp.asarray(a))

    def _A_setup():
        B, H, Sq, Sk, D, M = (1, 32, 2048, 2048, 128, 576)
        Dc = 4 * D
        return {'x': _w((lambda *s: _rng.normal(s) * 0.05)(B, Sq, M)), 'c_kv': _w((lambda *s: _rng.normal(s) * 0.05)(B, Sk, Dc)), 'w_q': _w((lambda *s: _rng.normal(s) * 0.05)(M, H, D) * M ** (-0.5)), 'w_uk': _w((lambda *s: _rng.normal(s) * 0.05)(Dc, H, D) * Dc ** (-0.5)), 'w_uv': _w((lambda *s: _rng.normal(s) * 0.05)(Dc, H, D) * Dc ** (-0.5)), 'w_o': _w((lambda *s: _rng.normal(s) * 0.05)(H, D, M) * (H * D) ** (-0.5))}
    _A_in = _A_setup()

    def _B_setup():
        B, S, Dm = (1, 2048, 576)
        H, Dh = (32, 128)
        M, seg = (8, 32)
        seg = min(seg, S)
        S = S // seg * seg
        return {'x': _w((lambda *s: _rng.normal(s) * 0.05)(B, S, Dm)), 'mem0': _w((lambda *s: _rng.normal(s) * 0.05)(B, M, Dm)), 'Wq': _w((lambda *s: _rng.normal(s) * 0.05)(Dm, H, Dh) * Dm ** (-0.5)), 'Wk': _w((lambda *s: _rng.normal(s) * 0.05)(Dm, H, Dh) * Dm ** (-0.5)), 'Wv': _w((lambda *s: _rng.normal(s) * 0.05)(Dm, H, Dh) * Dm ** (-0.5)), 'Wo': _w((lambda *s: _rng.normal(s) * 0.05)(H, Dh, Dm) * (H * Dh) ** (-0.5)), 'seg_len': seg}
    _B_in = _B_setup()
    return {'A_x': _A_in['x'], 'A_c_kv': _A_in['c_kv'], 'A_w_q': _A_in['w_q'], 'A_w_uk': _A_in['w_uk'], 'A_w_uv': _A_in['w_uv'], 'A_w_o': _A_in['w_o'], 'B_x': _B_in['x'], 'B_mem0': _B_in['mem0'], 'B_Wq': _B_in['Wq'], 'B_Wk': _B_in['Wk'], 'B_Wv': _B_in['Wv'], 'B_Wo': _B_in['Wo'], 'B_seg_len': _B_in['seg_len']}

def reference(A_x, A_c_kv, A_w_q, A_w_uk, A_w_uv, A_w_o, B_x, B_mem0, B_Wq, B_Wk, B_Wv, B_Wo, B_seg_len):

    def _A_ref(x, c_kv, w_q, w_uk, w_uv, w_o):
        B, Sq, M = (x.shape[0], x.shape[1], x.shape[2])
        Sk = c_kv.shape[1]
        H, D = (w_q.shape[1], w_q.shape[2])
        q = jnp.einsum('bqm,mhd->bhqd', x, w_q)
        k = jnp.einsum('bkc,chd->bhkd', c_kv, w_uk)
        v = jnp.einsum('bkc,chd->bhkd', c_kv, w_uv)
        scores = jnp.einsum('bhqd,bhkd->bhqk', q, k) * D ** (-0.5)
        off = Sk - Sq
        qi = jnp.arange(Sq)[:, None]
        kj = jnp.arange(Sk)[None, :]
        cmask = kj <= qi + off
        scores = jnp.where(cmask[None, None], scores, -1000000000.0)
        p = _softmax(scores, axis=-1)
        ctx = jnp.einsum('bhqk,bhkd->bhqd', p, v)
        return jnp.einsum('bhqd,hdm->bqm', ctx, w_o)

    def _B_ref(x, mem0, Wq, Wk, Wv, Wo, seg_len):
        B, S, Dm = x.shape
        H, Dh = (Wq.shape[1], Wq.shape[2])
        M = mem0.shape[1]
        scale = Dh ** (-0.5)
        n_seg = S // seg_len
        L = M + seg_len
        idx = jnp.arange(L)
        mask = (idx[:, None] < M) | (idx[:, None] >= idx[None, :])
        mem = mem0
        outs = []
        for s in range(n_seg):
            xs = x[:, s * seg_len:(s + 1) * seg_len, :].copy()
            h = jnp.concatenate([mem, xs], axis=1)
            q = jnp.einsum('btd,dhe->bhte', h, Wq)
            k = jnp.einsum('btd,dhe->bhte', h, Wk)
            v = jnp.einsum('btd,dhe->bhte', h, Wv)
            scores = jnp.einsum('bhqe,bhke->bhqk', q, k) * scale
            scores = jnp.where(mask[None, None], scores, -1000000000.0)
            p = _softmax(scores, axis=-1)
            o = jnp.einsum('bhqk,bhke->bhqe', p, v)
            o = jnp.einsum('bhte,hed->btd', o, Wo)
            mem = o[:, :M, :].copy()
            outs.append(o[:, M:, :])
        return jnp.concatenate(outs, axis=1)
    a = _A_ref(A_x, A_c_kv, A_w_q, A_w_uk, A_w_uv, A_w_o)
    b = _B_ref(B_x, B_mem0, B_Wq, B_Wk, B_Wv, B_Wo, B_seg_len)
    return jnp.concatenate([a, b], axis=-1)
```

```python
import functools

import jax
import jax.numpy as jnp
from jax.experimental import pallas as pl
from jax.experimental.pallas import tpu as pltpu

_LOG2E = 1.4426950408889634
_NT = (((1,), (1,)), ((), ()))
_NEG = -1e30
_BF = jnp.bfloat16
_F32 = jnp.float32


def _dot(a, b):
    return jnp.dot(a, b, preferred_element_type=_F32)


def _dot_nt(a, b):
    return jax.lax.dot_general(a, b, _NT, preferred_element_type=_F32)


def _rcp(l):
    r = pltpu.reciprocal(l, approx=True)
    return r * (2.0 - l * r)


def _relayout(src_ref, dst_ref, rows=64):
    k, h, d = src_ref.shape
    for k0 in range(0, k, rows):
        dst_ref[k0:k0 + rows, :] = src_ref[k0:k0 + rows, :, :].reshape(rows, h * d)


def _transpose_into(src_ref, dst_ref, cols=256):
    for c0 in range(0, src_ref.shape[1], cols):
        dst_ref[c0:c0 + cols, :] = src_ref[:, c0:c0 + cols].T


def _wo_into(src_ref, dst_ref):
    h, _, d = src_ref.shape
    for hh in range(h):
        dst_ref[hh * d:(hh + 1) * d, :] = src_ref[hh].T


def _a_head(h, x_v, c_v, wq, wk, wv, q_s, k_s, v_s, s_scr, ctx, S, D, bq):
    col = pl.ds(pl.multiple_of(h * D, D), D)
    scale = (D ** -0.5) * _LOG2E
    q_s[...] = (_dot(x_v[...], wq[:, col]) * scale).astype(_BF)
    k_s[...] = _dot(c_v[...], wk[:, col]).astype(_BF)
    v_s[...] = _dot(c_v[...], wv[:, col]).astype(_BF)
    nb = S // bq
    order = []
    lo, hi = 0, nb - 1
    while lo <= hi:
        order.append(hi)
        if lo != hi:
            order.append(lo)
        lo += 1
        hi -= 1
    r = jax.lax.broadcasted_iota(jnp.int32, (bq, bq), 0)
    c = jax.lax.broadcasted_iota(jnp.int32, (bq, bq), 1)
    tri = c <= r
    ms = {}
    for t in range(nb + 1):
        if t < nb:
            qi = order[t]
            L = (qi + 1) * bq
            s = _dot_nt(q_s[qi * bq:L, :], k_s[0:L, :])
            sd = jnp.where(tri, s[:, L - bq:], _NEG)
            s = jnp.concatenate([s[:, :L - bq], sd], axis=1) if L > bq else sd
            ms[t] = jnp.max(s, axis=1, keepdims=True)
            s_scr[t % 2, :, 0:L] = s
        if t > 0:
            qi = order[t - 1]
            L = (qi + 1) * bq
            p = jnp.exp2(s_scr[(t - 1) % 2, :, 0:L] - ms.pop(t - 1))
            l = jnp.sum(p, axis=1, keepdims=True)
            o = _dot(p.astype(_BF), v_s[0:L, :])
            ctx[qi * bq:L, col] = (o * _rcp(l)).astype(_BF)


def _b_attend(q, k, v, ok, H, D, scale):
    outs = []
    for hh in range(H):
        sl = slice(hh * D, (hh + 1) * D)
        qh = (q[:, sl] * scale).astype(_BF)
        kh = k[:, sl].astype(_BF)
        vh = v[:, sl].astype(_BF)
        sc = jnp.where(ok, _dot_nt(qh, kh), _NEG)
        m = jnp.max(sc, axis=1, keepdims=True)
        p = jnp.exp2(sc - m)
        l = jnp.sum(p, axis=1, keepdims=True)
        p = p * _rcp(l)
        outs.append(_dot(p.astype(_BF), vh))
    return jnp.concatenate(outs, axis=1)


def _b_pair(i, mem, bx, wq, wk, wv, wo, out_v, H, D, DM):
    scale = (D ** -0.5) * _LOG2E
    row0 = pl.multiple_of(i * 64, 64)
    xa = bx[pl.ds(row0, 32), :]
    xb = bx[pl.ds(row0 + 32, 32), :].astype(_F32)
    r = jax.lax.broadcasted_iota(jnp.int32, (48, 48), 0)
    c = jax.lax.broadcasted_iota(jnp.int32, (48, 48), 1)
    ok = (c < 40) & ((r >= 32) | (c >= 32) | (c <= r))

    ha = jnp.concatenate([xa, jnp.concatenate([mem, xb[0:8]], axis=0).astype(_BF)], axis=0)
    qa = _dot(ha, wq[...])
    ka = _dot(ha, wk[...])
    va = _dot(ha, wv[...])
    oa = _b_attend(qa, ka, va, ok, H, D, scale)
    la = jnp.concatenate([oa[0:24], oa[32:40]], axis=0).astype(_BF)
    ra = _dot(la, wo[...])
    mem_b = ra[24:32].astype(_BF).astype(_F32)

    hb = jnp.concatenate([xb[8:32], mem_b], axis=0).astype(_BF)
    qb = _dot(hb, wq[...])
    kb = _dot(hb, wk[...])
    vb = _dot(hb, wv[...])
    asm = lambda first, rest: jnp.concatenate([first[40:48], rest, rest[24:32]], axis=0)
    ob = _b_attend(asm(qa, qb), asm(ka, kb), asm(va, vb), ok, H, D, scale)
    lb = jnp.concatenate([oa[24:32], ob[0:40]], axis=0).astype(_BF)
    rb = _dot(lb, wo[...])
    res = jnp.concatenate([ra[0:24], rb[0:40]], axis=0).astype(_BF)
    out_v[pl.ds(row0, 64), DM:2 * DM] = res
    return rb[40:48].astype(_BF).astype(_F32)


def _kernel(axt_h, ac_h, awq_h, awk_h, awv_h, awo_h, bxt_h, bm_h, bwq_h, bwk_h, bwv_h, bwo_h,
            out_h,
            ax, ac, bx, bm, raw0, raw1, raw2, awq, awk, awv, awo, bwq, bwk, bwv, bwo,
            q_s, k_s, v_s, s_scr, ctx, out_v, xt_s, wo_raw, sems):
    S, DM = ax.shape
    DC = ac.shape[1]
    H, D = awq_h.shape[1], awq_h.shape[2]

    def cp(i, src, dst):
        return pltpu.make_async_copy(src, dst, sems.at[i])

    c_wq = cp(0, awq_h, raw0.at[0:DM])
    c_x = cp(1, axt_h, xt_s)
    c_wk = cp(2, awk_h, raw1.at[0:DC])
    c_c = cp(3, ac_h, ac)
    c_wv = cp(4, awv_h, raw2.at[0:DC])
    c_wo = cp(5, awo_h, wo_raw)
    c_bm = cp(7, bm_h, bm)
    for c in (c_x, c_wq, c_wk, c_c, c_wv, c_wo, c_bm):
        c.start()
    c_x.wait()
    _transpose_into(xt_s, ax)
    c_bx = cp(6, bxt_h, xt_s)
    c_bx.start()
    c_wq.wait()
    _relayout(raw0.at[0:DM], awq)
    c_wk.wait()
    _relayout(raw1.at[0:DC], awk)
    c_wv.wait()
    _relayout(raw2.at[0:DC], awv)
    c_bq = cp(9, bwq_h, raw0)
    c_bk = cp(10, bwk_h, raw1)
    c_bv = cp(11, bwv_h, raw2)
    c_bq.start()
    c_bk.start()
    c_bv.start()
    c_wo.wait()
    _wo_into(wo_raw, awo)
    c_bwo = cp(8, bwo_h, wo_raw)
    c_bwo.start()
    c_c.wait()

    def a_body(h, carry):
        _a_head(h, ax, ac, awq, awk, awv, q_s, k_s, v_s, s_scr, ctx, S, D, 128)
        return carry

    jax.lax.fori_loop(0, H, a_body, 0)

    def ao_body(i, carry):
        rows = pl.ds(pl.multiple_of(i * 256, 256), 256)
        out_v[rows, 0:DM] = _dot(ctx[rows, :], awo[...]).astype(_BF)
        return carry

    jax.lax.fori_loop(0, S // 256, ao_body, 0)

    c_bq.wait()
    _relayout(raw0, bwq)
    c_bk.wait()
    _relayout(raw1, bwk)
    c_bv.wait()
    _relayout(raw2, bwv)
    c_bx.wait()
    _transpose_into(xt_s, bx)
    c_bm.wait()
    c_bwo.wait()
    _wo_into(wo_raw, bwo)

    def b_body(i, mem):
        return _b_pair(i, mem, bx, bwq, bwk, bwv, bwo, out_v, H, D, DM)

    jax.lax.fori_loop(0, S // 64, b_body, bm[...].astype(_F32))

    c_out = cp(12, out_v, out_h)
    c_out.start()
    c_out.wait()


@functools.partial(jax.jit, static_argnames=("B_seg_len",))
def pallas_concat_heads__compressed_kv_cla__memory_aug_recurrent_mem_tr__prompt_kernel(
        A_x, A_c_kv, A_w_q, A_w_uk, A_w_uv, A_w_o,
        B_x, B_mem0, B_Wq, B_Wk, B_Wv, B_Wo, B_seg_len):
    _, S, DM = A_x.shape
    DC = A_c_kv.shape[2]
    H, D = A_w_q.shape[1], A_w_q.shape[2]
    M = B_mem0.shape[1]
    assert B_seg_len == 32 and M == 8 and B_x.shape[1] == S

    any_spec = pl.BlockSpec(memory_space=pl.ANY)
    vm = lambda shape, dt=_BF: pltpu.VMEM(shape, dt)
    out = pl.pallas_call(
        _kernel,
        out_shape=jax.ShapeDtypeStruct((S, 2 * DM), _BF),
        in_specs=[any_spec] * 12,
        out_specs=any_spec,
        scratch_shapes=[
            vm((S, DM)), vm((S, DC)), vm((S, DM)), vm((M, DM)),
            vm((DM, H, D)), vm((DM, H, D)), vm((DM, H, D)),
            vm((DM, H * D)), vm((DC, H * D)), vm((DC, H * D)), vm((H * D, DM)),
            vm((DM, H * D)), vm((DM, H * D)), vm((DM, H * D)), vm((H * D, DM)),
            vm((S, D)), vm((S, D)), vm((S, D)), vm((2, 128, S), _F32),
            vm((S, H * D)), vm((S, 2 * DM)), vm((DM, S)), vm((H, DM, D)),
            pltpu.SemaphoreType.DMA((13,)),
        ],
        compiler_params=pltpu.CompilerParams(vmem_limit_bytes=120 * 1024 * 1024),
    )(
        A_x.reshape(S, DM).T, A_c_kv.reshape(S, DC), A_w_q, A_w_uk, A_w_uv,
        jnp.swapaxes(A_w_o, 1, 2),
        B_x.reshape(S, DM).T, B_mem0.reshape(M, DM), B_Wq, B_Wk, B_Wv,
        jnp.swapaxes(B_Wo, 1, 2),
    )
    return out.reshape(1, S, 2 * DM)
```

```python
import functools

import jax
import jax.numpy as jnp
from jax.experimental import pallas as pl
from jax.experimental.pallas import tpu as pltpu

_LOG2E = 1.4426950408889634
_NT = (((1,), (1,)), ((), ()))
_NEG = -1e30
_BF = jnp.bfloat16
_F32 = jnp.float32


def _dot(a, b):
    return jnp.dot(a, b, preferred_element_type=_F32)


def _dot_nt(a, b):
    return jax.lax.dot_general(a, b, _NT, preferred_element_type=_F32)


def _rcp(l):
    r = pltpu.reciprocal(l, approx=True)
    return r * (2.0 - l * r)


def _relayout(src_ref, dst_ref, rows=64):
    k, h, d = src_ref.shape
    for k0 in range(0, k, rows):
        dst_ref[k0:k0 + rows, :] = src_ref[k0:k0 + rows, :, :].reshape(rows, h * d)


def _transpose_into(src_ref, dst_ref, cols=256):
    for c0 in range(0, src_ref.shape[1], cols):
        dst_ref[c0:c0 + cols, :] = src_ref[:, c0:c0 + cols].T


def _wo_into(src_ref, dst_ref):
    h, _, d = src_ref.shape
    for hh in range(h):
        dst_ref[hh * d:(hh + 1) * d, :] = src_ref[hh].T


def _a_head(h, x_v, c_v, wq, wk, wv, q_s, k_s, v_s, s_scr, ctx, S, D, bq):
    col = pl.ds(pl.multiple_of(h * D, D), D)
    scale = (D ** -0.5) * _LOG2E
    k_s[...] = _dot(c_v[...], wk[:, col]).astype(_BF)
    yield 2048
    q_s[...] = (_dot(x_v[...], wq[:, col]) * scale).astype(_BF)
    yield 2560
    v_s[...] = _dot(c_v[...], wv[:, col]).astype(_BF)
    yield 2048
    nb = S // bq
    order = []
    lo, hi = 0, nb - 1
    while lo <= hi:
        order.append(hi)
        if lo != hi:
            order.append(lo)
        lo += 1
        hi -= 1
    r = jax.lax.broadcasted_iota(jnp.int32, (bq, bq), 0)
    c = jax.lax.broadcasted_iota(jnp.int32, (bq, bq), 1)
    tri = c <= r
    ms = {}
    for t in range(nb + 1):
        if t < nb:
            qi = order[t]
            L = (qi + 1) * bq
            s = _dot_nt(q_s[qi * bq:L, :], k_s[0:L, :])
            sd = jnp.where(tri, s[:, L - bq:], _NEG)
            s = jnp.concatenate([s[:, :L - bq], sd], axis=1) if L > bq else sd
            ms[t] = jnp.max(s, axis=1, keepdims=True)
            s_scr[t % 2, :, 0:L] = s
            yield (qi + 1) * 32
        if t > 0:
            qi = order[t - 1]
            L = (qi + 1) * bq
            p = jnp.exp2(s_scr[(t - 1) % 2, :, 0:L] - ms.pop(t - 1))
            l = jnp.sum(p, axis=1, keepdims=True)
            o = _dot(p.astype(_BF), v_s[0:L, :])
            ctx[qi * bq:L, col] = (o * _rcp(l)).astype(_BF)
            yield (qi + 1) * 32


def _b_seg(h_in, asm, sel, wq, wk, wv, wo, ok, H, D, G):
    scale = (D ** -0.5) * _LOG2E
    NG = H // G
    qkv, pv, og = {}, {}, {}
    acc = None
    for t in range(NG + 3):
        if t < NG:
            sl = slice(t * G * D, (t + 1) * G * D)
            qkv[t] = (_dot(h_in, wq[:, sl]), _dot(h_in, wk[:, sl]), _dot(h_in, wv[:, sl]))
        g = t - 1
        if 0 <= g < NG:
            q, k, v = qkv.pop(g)
            q, k, v = asm(0, g, q), asm(1, g, k), asm(2, g, v)
            items = []
            for hh in range(G):
                c = slice(hh * D, (hh + 1) * D)
                qh = (q[:, c] * scale).astype(_BF)
                kh = k[:, c].astype(_BF)
                sc = jnp.where(ok, _dot_nt(qh, kh), _NEG)
                m = jnp.max(sc, axis=1, keepdims=True)
                p = jnp.exp2(sc - m)
                l = jnp.sum(p, axis=1, keepdims=True)
                items.append(((p * _rcp(l)).astype(_BF), v[:, c].astype(_BF)))
            pv[g] = items
        g = t - 2
        if 0 <= g < NG:
            og[g] = sel(g, jnp.concatenate([_dot(p, vh) for p, vh in pv.pop(g)], axis=1))
        g = t - 3
        if 0 <= g < NG:
            r = _dot(og.pop(g), wo[g * G * D:(g + 1) * G * D, :])
            acc = r if acc is None else acc + r
    return acc


def _b_pair(i, mem, bx, wq, wk, wv, wo, out_v, H, D, DM, res_out, G=4):
    row0 = pl.multiple_of(i * 64, 64)
    xa = bx[pl.ds(row0, 32), :]
    xb = bx[pl.ds(row0 + 32, 32), :].astype(_F32)
    r = jax.lax.broadcasted_iota(jnp.int32, (48, 48), 0)
    c = jax.lax.broadcasted_iota(jnp.int32, (48, 48), 1)
    ok = (c < 40) & ((r >= 32) | (c >= 32) | (c <= r))

    ha = jnp.concatenate([xa, jnp.concatenate([mem, xb[0:8]], axis=0).astype(_BF)], axis=0)
    saved, o_tail = {}, {}

    def asm_a(n, g, val):
        saved[(n, g)] = val[40:48]
        return val

    def sel_a(g, o):
        o_tail[g] = o[24:32]
        return jnp.concatenate([o[0:24], o[32:40]], axis=0).astype(_BF)

    ra = _b_seg(ha, asm_a, sel_a, wq, wk, wv, wo, ok, H, D, G)
    yield
    ra = ra
    mem_b = ra[24:32].astype(_BF).astype(_F32)

    hb = jnp.concatenate([xb[8:32], mem_b], axis=0).astype(_BF)

    def asm_b(n, g, val):
        return jnp.concatenate([saved.pop((n, g)), val, val[24:32]], axis=0)

    def sel_b(g, o):
        return jnp.concatenate([o_tail.pop(g), o[0:40]], axis=0).astype(_BF)

    rb = _b_seg(hb, asm_b, sel_b, wq, wk, wv, wo, ok, H, D, G)
    rb = rb
    res = jnp.concatenate([ra[0:24], rb[0:40]], axis=0).astype(_BF)
    out_v[pl.ds(row0, 64), DM:2 * DM] = res
    res_out["mem"] = rb[40:48].astype(_BF).astype(_F32)


def _drain(gen):
    for _ in gen:
        pass


def _kernel(axt_h, ac_h, awq_h, awk_h, awv_h, awo_h, bxt_h, bm_h, bwq_h, bwk_h, bwv_h, bwo_h,
            out_h,
            ax, ac, bx, bm, raw0, raw1, raw2, awq, awk, awv, awo, bwq, bwk, bwv, bwo,
            q_s, k_s, v_s, s_scr, ctx, out_v, xt_s, wo_raw, braw, sems, bsems, osems):
    S, DM = ax.shape
    DC = ac.shape[1]
    H, D = awq_h.shape[1], awq_h.shape[2]
    NA = 4
    KS = DM // NA
    XS = S // NA
    HS = H // NA
    OS = S // NA

    def cp(i, src, dst):
        return pltpu.make_async_copy(src, dst, sems.at[i])

    def bcp(w, i):
        src = (bwq_h, bwk_h, bwv_h)[w]
        rows = pl.ds(pl.multiple_of(i * KS, 16), KS)
        return pltpu.make_async_copy(src.at[rows], braw.at[w, rows], bsems.at[w * NA + i])

    def ocp(j):
        rows = pl.ds(pl.multiple_of(j * OS, OS), OS)
        return pltpu.make_async_copy(out_v.at[rows], out_h.at[rows], osems.at[j])

    c_x = cp(1, axt_h, xt_s)
    c_wq = cp(0, awq_h, raw0.at[0:DM])
    c_wk = cp(2, awk_h, raw1.at[0:DC])
    c_c = cp(3, ac_h, ac)
    c_wv = cp(4, awv_h, raw2.at[0:DC])
    c_bm = cp(7, bm_h, bm)
    c_bwo = cp(8, bwo_h, wo_raw)
    for c in (c_x, c_wq, c_wk, c_c, c_wv):
        c.start()
    c_x.wait()
    _transpose_into(xt_s, ax)
    c_wq.wait()
    _relayout(raw0.at[0:DM], awq)
    c_wk.wait()
    _relayout(raw1.at[0:DC], awk)
    c_wv.wait()
    c_c.wait()
    c_bx = cp(6, bxt_h, xt_s)
    for i in range(NA):
        for w in range(3):
            bcp(w, i).start()
    c_bx.start()
    c_bm.start()
    c_bwo.start()
    _relayout(raw2.at[0:DC], awv)

    def a_gen(h):
        return _a_head(h, ax, ac, awq, awk, awv, q_s, k_s, v_s, s_scr, ctx, S, D, 128)

    def warm_body(i, carry):
        ga = a_gen(i)
        next(ga)
        for w, dst in enumerate((bwq, bwk, bwv)):
            bcp(w, i).wait()
            for r0 in range(0, KS, 48):
                rows = pl.ds(pl.multiple_of(i * KS + r0, 16), 48)
                dst[rows, :] = braw[w, rows, :, :].reshape(48, H * D)
            next(ga)
        _drain(ga)
        return carry

    jax.lax.fori_loop(0, NA, warm_body, 0)
    c_bx.wait()
    _transpose_into(xt_s, bx)
    c_bm.wait()
    c_bwo.wait()
    _wo_into(wo_raw, bwo)
    c_wo = cp(5, awo_h, wo_raw)
    c_wo.start()

    def ab_body(i, mem):
        res = {}
        ga = a_gen(i + NA)
        gb = _b_pair(i, mem, bx, bwq, bwk, bwv, bwo, out_v, H, D, DM, res)
        next(ga)
        next(gb)
        next(ga)
        _drain(gb)
        _drain(ga)
        return res["mem"]

    mem = jax.lax.fori_loop(0, H - NA, ab_body, bm[...].astype(_F32))
    c_wo.wait()
    _wo_into(wo_raw, awo)

    def tail_body(j, mem):
        res = {}
        gb = _b_pair(j + H - NA, mem, bx, bwq, bwk, bwv, bwo, out_v, H, D, DM, res)

        def oproj(r0):
            rows = pl.ds(pl.multiple_of(j * OS + r0, 256), 256)
            out_v[rows, 0:DM] = _dot(ctx[rows, :], awo[...]).astype(_BF)

        oproj(0)
        next(gb)
        oproj(256)
        _drain(gb)

        @pl.when(j > 0)
        def _():
            ocp(j - 1).start()

        return res["mem"]

    jax.lax.fori_loop(0, NA, tail_body, mem)
    ocp(NA - 1).start()
    for j in range(NA):
        ocp(j).wait()


@functools.partial(jax.jit, static_argnames=("B_seg_len",))
def pallas_concat_heads__compressed_kv_cla__memory_aug_recurrent_mem_tr__prompt_kernel(
        A_x, A_c_kv, A_w_q, A_w_uk, A_w_uv, A_w_o,
        B_x, B_mem0, B_Wq, B_Wk, B_Wv, B_Wo, B_seg_len):
    _, S, DM = A_x.shape
    DC = A_c_kv.shape[2]
    H, D = A_w_q.shape[1], A_w_q.shape[2]
    M = B_mem0.shape[1]
    assert B_seg_len == 32 and M == 8 and B_x.shape[1] == S

    any_spec = pl.BlockSpec(memory_space=pl.ANY)
    vm = lambda shape, dt=_BF: pltpu.VMEM(shape, dt)
    out = pl.pallas_call(
        _kernel,
        out_shape=jax.ShapeDtypeStruct((S, 2 * DM), _BF),
        in_specs=[any_spec] * 12,
        out_specs=any_spec,
        scratch_shapes=[
            vm((S, DM)), vm((S, DC)), vm((S, DM)), vm((M, DM)),
            vm((DM, H, D)), vm((DM, H, D)), vm((DM, H, D)),
            vm((DM, H * D)), vm((DC, H * D)), vm((DC, H * D)), vm((H * D, DM)),
            vm((DM, H * D)), vm((DM, H * D)), vm((DM, H * D)), vm((H * D, DM)),
            vm((S, D)), vm((S, D)), vm((S, D)), vm((2, 128, S), _F32),
            vm((S, H * D)), vm((S, 2 * DM)), vm((DM, S)), vm((H, DM, D)),
            vm((3, DM, H, D)),
            pltpu.SemaphoreType.DMA((9,)), pltpu.SemaphoreType.DMA((12,)),
            pltpu.SemaphoreType.DMA((4,)),
        ],
        compiler_params=pltpu.CompilerParams(vmem_limit_bytes=120 * 1024 * 1024),
    )(
        A_x.reshape(S, DM).T, A_c_kv.reshape(S, DC), A_w_q, A_w_uk, A_w_uv,
        jnp.swapaxes(A_w_o, 1, 2),
        B_x.reshape(S, DM).T, B_mem0.reshape(M, DM), B_Wq, B_Wk, B_Wv,
        jnp.swapaxes(B_Wo, 1, 2),
    )
    return out.reshape(1, S, 2 * DM)
```

```python
import functools

import jax
import jax.numpy as jnp
from jax.experimental import pallas as pl
from jax.experimental.pallas import tpu as pltpu

_LOG2E = 1.4426950408889634
_NT = (((1,), (1,)), ((), ()))
_NEG = -1e30
_BF = jnp.bfloat16
_F32 = jnp.float32


def _dot(a, b):
    return jnp.dot(a, b, preferred_element_type=_F32)


def _dot_nt(a, b):
    return jax.lax.dot_general(a, b, _NT, preferred_element_type=_F32)


def _rcp(l):
    r = pltpu.reciprocal(l, approx=True)
    return r * (2.0 - l * r)


def _relayout(src_ref, dst_ref, rows=64):
    k, h, d = src_ref.shape
    for k0 in range(0, k, rows):
        dst_ref[k0:k0 + rows, :] = src_ref[k0:k0 + rows, :, :].reshape(rows, h * d)


def _transpose_into(src_ref, dst_ref, cols=256):
    for c0 in range(0, src_ref.shape[1], cols):
        dst_ref[c0:c0 + cols, :] = src_ref[:, c0:c0 + cols].T


def _wo_into(src_ref, dst_ref):
    h, _, d = src_ref.shape
    for hh in range(h):
        dst_ref[hh * d:(hh + 1) * d, :] = src_ref[hh].T


def _a_head(h, x_v, c_v, wq, wk, wv, q_s, k_s, v_s, s_scr, ctx, S, D, bq, pc):
    col = pl.ds(pl.multiple_of(h * D, D), D)
    scale = (D ** -0.5) * _LOG2E
    for r0 in range(0, S, pc):
        k_s[r0:r0 + pc, :] = _dot(c_v[r0:r0 + pc, :], wk[:, col]).astype(_BF)
        yield
    for r0 in range(0, S, pc):
        q_s[r0:r0 + pc, :] = (_dot(x_v[r0:r0 + pc, :], wq[:, col]) * scale).astype(_BF)
        yield
    for r0 in range(0, S, pc):
        v_s[r0:r0 + pc, :] = _dot(c_v[r0:r0 + pc, :], wv[:, col]).astype(_BF)
        yield
    nb = S // bq
    order = []
    lo, hi = 0, nb - 1
    while lo <= hi:
        order.append(hi)
        if lo != hi:
            order.append(lo)
        lo += 1
        hi -= 1
    r = jax.lax.broadcasted_iota(jnp.int32, (bq, bq), 0)
    c = jax.lax.broadcasted_iota(jnp.int32, (bq, bq), 1)
    tri = c <= r
    ms = {}
    for t in range(nb + 1):
        if t < nb:
            qi = order[t]
            L = (qi + 1) * bq
            s = _dot_nt(q_s[qi * bq:L, :], k_s[0:L, :])
            sd = jnp.where(tri, s[:, L - bq:], _NEG)
            s = jnp.concatenate([s[:, :L - bq], sd], axis=1) if L > bq else sd
            ms[t] = jnp.max(s, axis=1, keepdims=True)
            s_scr[t % 2, :, 0:L] = s
            yield (qi + 1) * 32
        if t > 0:
            qi = order[t - 1]
            L = (qi + 1) * bq
            p = jnp.exp2(s_scr[(t - 1) % 2, :, 0:L] - ms.pop(t - 1))
            l = jnp.sum(p, axis=1, keepdims=True)
            o = _dot(p.astype(_BF), v_s[0:L, :])
            ctx[qi * bq:L, col] = (o * _rcp(l)).astype(_BF)
            yield (qi + 1) * 32


def _b_seg(h_in, asm, sel, wq, wk, wv, wo, ok, H, D, G):
    scale = (D ** -0.5) * _LOG2E
    NG = H // G
    qkv, pv, og = {}, {}, {}
    acc = None
    for t in range(NG + 3):
        if t < NG:
            sl = slice(t * G * D, (t + 1) * G * D)
            qkv[t] = (_dot(h_in, wq[:, sl]), _dot(h_in, wk[:, sl]), _dot(h_in, wv[:, sl]))
        g = t - 1
        if 0 <= g < NG:
            q, k, v = qkv.pop(g)
            q, k, v = asm(0, g, q), asm(1, g, k), asm(2, g, v)
            items = []
            for hh in range(G):
                c = slice(hh * D, (hh + 1) * D)
                qh = (q[:, c] * scale).astype(_BF)
                kh = k[:, c].astype(_BF)
                sc = jnp.where(ok, _dot_nt(qh, kh), _NEG)
                m = jnp.max(sc, axis=1, keepdims=True)
                p = jnp.exp2(sc - m)
                l = jnp.sum(p, axis=1, keepdims=True)
                items.append(((p * _rcp(l)).astype(_BF), v[:, c].astype(_BF)))
            pv[g] = items
        g = t - 2
        if 0 <= g < NG:
            og[g] = sel(g, jnp.concatenate([_dot(p, vh) for p, vh in pv.pop(g)], axis=1))
        g = t - 3
        if 0 <= g < NG:
            r = _dot(og.pop(g), wo[g * G * D:(g + 1) * G * D, :])
            acc = r if acc is None else acc + r
    return acc


def _b_pair(i, mem, bx, wq, wk, wv, wo, out_v, H, D, DM, res_out, G=4):
    row0 = pl.multiple_of(i * 64, 64)
    xa = bx[pl.ds(row0, 32), :]
    xb = bx[pl.ds(row0 + 32, 32), :].astype(_F32)
    r = jax.lax.broadcasted_iota(jnp.int32, (48, 48), 0)
    c = jax.lax.broadcasted_iota(jnp.int32, (48, 48), 1)
    ok = (c < 40) & ((r >= 32) | (c >= 32) | (c <= r))

    ha = jnp.concatenate([xa, jnp.concatenate([mem, xb[0:8]], axis=0).astype(_BF)], axis=0)
    saved, o_tail = {}, {}

    def asm_a(n, g, val):
        saved[(n, g)] = val[40:48]
        return val

    def sel_a(g, o):
        o_tail[g] = o[24:32]
        return jnp.concatenate([o[0:24], o[32:40]], axis=0).astype(_BF)

    ra = _b_seg(ha, asm_a, sel_a, wq, wk, wv, wo, ok, H, D, G)
    yield
    ra = ra
    mem_b = ra[24:32].astype(_BF).astype(_F32)

    hb = jnp.concatenate([xb[8:32], mem_b], axis=0).astype(_BF)

    def asm_b(n, g, val):
        return jnp.concatenate([saved.pop((n, g)), val, val[24:32]], axis=0)

    def sel_b(g, o):
        return jnp.concatenate([o_tail.pop(g), o[0:40]], axis=0).astype(_BF)

    rb = _b_seg(hb, asm_b, sel_b, wq, wk, wv, wo, ok, H, D, G)
    rb = rb
    res = jnp.concatenate([ra[0:24], rb[0:40]], axis=0).astype(_BF)
    out_v[pl.ds(row0, 64), DM:2 * DM] = res
    res_out["mem"] = rb[40:48].astype(_BF).astype(_F32)


def _advance(gen, n):
    for _ in range(n):
        next(gen)


def _drain(gen):
    for _ in gen:
        pass


def _kernel(axt_h, ac_h, awq_h, awk_h, awv_h, awo_h, bxt_h, bm_h, bwq_h, bwk_h, bwv_h, bwo_h,
            out_h,
            ax, ac, bx, bm, raw0, raw1, raw2, awq, awk, awv, awo, bwq, bwk, bwv, bwo,
            q_s, k_s, v_s, s_scr, ctx, out_v, xt_s, wo_raw, braw, sems, bsems, osems):
    S, DM = ax.shape
    DC = ac.shape[1]
    H, D = awq_h.shape[1], awq_h.shape[2]
    NA = 4
    KS = DM // NA
    XS = S // NA
    HS = H // NA
    OS = S // NA

    def cp(i, src, dst):
        return pltpu.make_async_copy(src, dst, sems.at[i])

    def bcp(w, i):
        src = (bwq_h, bwk_h, bwv_h)[w]
        rows = pl.ds(pl.multiple_of(i * KS, 16), KS)
        return pltpu.make_async_copy(src.at[rows], braw.at[w, rows], bsems.at[w * NA + i])

    def ocp(j):
        rows = pl.ds(pl.multiple_of(j * OS, OS), OS)
        return pltpu.make_async_copy(out_v.at[rows], out_h.at[rows], osems.at[j])

    c_x = cp(1, axt_h, xt_s)
    c_wq = cp(0, awq_h, raw0.at[0:DM])
    c_wk = cp(2, awk_h, raw1.at[0:DC])
    c_c = cp(3, ac_h, ac)
    c_wv = cp(4, awv_h, raw2.at[0:DC])
    c_bm = cp(7, bm_h, bm)
    c_bwo = cp(8, bwo_h, wo_raw)
    for c in (c_x, c_wq, c_wk, c_c, c_wv):
        c.start()
    c_x.wait()
    _transpose_into(xt_s, ax)
    c_wq.wait()
    _relayout(raw0.at[0:DM], awq)
    c_wk.wait()
    _relayout(raw1.at[0:DC], awk)
    c_wv.wait()
    c_c.wait()
    c_bx = cp(6, bxt_h, xt_s)
    for i in range(NA):
        for w in range(3):
            bcp(w, i).start()
    c_bx.start()
    c_bm.start()
    c_bwo.start()
    _relayout(raw2.at[0:DC], awv)

    def a_gen(h, pc=512):
        return _a_head(h, ax, ac, awq, awk, awv, q_s, k_s, v_s, s_scr, ctx, S, D, 128, pc)

    def warm_body(i, carry):
        ga = a_gen(i, 128)
        next(ga)
        for w, dst in enumerate((bwq, bwk, bwv)):
            bcp(w, i).wait()
            for r0 in range(0, KS, 16):
                rows = pl.ds(pl.multiple_of(i * KS + r0, 16), 16)
                dst[rows, :] = braw[w, rows, :, :].reshape(16, H * D)
                next(ga)
        _drain(ga)
        return carry

    jax.lax.fori_loop(0, NA, warm_body, 0)
    c_bx.wait()
    _transpose_into(xt_s, bx)
    c_bm.wait()
    c_bwo.wait()
    _wo_into(wo_raw, bwo)
    c_wo = cp(5, awo_h, wo_raw)
    c_wo.start()

    def ab_body(i, mem):
        res = {}
        ga = a_gen(i + NA)
        gb = _b_pair(i, mem, bx, bwq, bwk, bwv, bwo, out_v, H, D, DM, res)
        _advance(ga, 4)
        next(gb)
        _advance(ga, 4)
        _drain(gb)
        _drain(ga)
        return res["mem"]

    mem = jax.lax.fori_loop(0, H - NA, ab_body, bm[...].astype(_F32))
    c_wo.wait()
    for hh in range(H):
        awo[:, hh * D:(hh + 1) * D] = wo_raw[hh]

    def tail_body(j, mem):
        res = {}
        gb = _b_pair(j + H - NA, mem, bx, bwq, bwk, bwv, bwo, out_v, H, D, DM, res)

        def oproj(r0):
            rows = pl.ds(pl.multiple_of(j * OS + r0, 256), 256)
            out_v[rows, 0:DM] = _dot_nt(awo[...], ctx[rows, :]).T.astype(_BF)

        oproj(0)
        next(gb)
        oproj(256)
        _drain(gb)

        @pl.when(j > 0)
        def _():
            ocp(j - 1).start()

        return res["mem"]

    jax.lax.fori_loop(0, NA, tail_body, mem)
    ocp(NA - 1).start()
    for j in range(NA):
        ocp(j).wait()


@functools.partial(jax.jit, static_argnames=("B_seg_len",))
def pallas_concat_heads__compressed_kv_cla__memory_aug_recurrent_mem_tr__prompt_kernel(
        A_x, A_c_kv, A_w_q, A_w_uk, A_w_uv, A_w_o,
        B_x, B_mem0, B_Wq, B_Wk, B_Wv, B_Wo, B_seg_len):
    _, S, DM = A_x.shape
    DC = A_c_kv.shape[2]
    H, D = A_w_q.shape[1], A_w_q.shape[2]
    M = B_mem0.shape[1]
    assert B_seg_len == 32 and M == 8 and B_x.shape[1] == S

    any_spec = pl.BlockSpec(memory_space=pl.ANY)
    vm = lambda shape, dt=_BF: pltpu.VMEM(shape, dt)
    out = pl.pallas_call(
        _kernel,
        out_shape=jax.ShapeDtypeStruct((S, 2 * DM), _BF),
        in_specs=[any_spec] * 12,
        out_specs=any_spec,
        scratch_shapes=[
            vm((S, DM)), vm((S, DC)), vm((S, DM)), vm((M, DM)),
            vm((DM, H, D)), vm((DM, H, D)), vm((DM, H, D)),
            vm((DM, H * D)), vm((DC, H * D)), vm((DC, H * D)), vm((DM, H * D)),
            vm((DM, H * D)), vm((DM, H * D)), vm((DM, H * D)), vm((H * D, DM)),
            vm((S, D)), vm((S, D)), vm((S, D)), vm((2, 128, S), _F32),
            vm((S, H * D)), vm((S, 2 * DM)), vm((DM, S)), vm((H, DM, D)),
            vm((3, DM, H, D)),
            pltpu.SemaphoreType.DMA((9,)), pltpu.SemaphoreType.DMA((12,)),
            pltpu.SemaphoreType.DMA((4,)),
        ],
        compiler_params=pltpu.CompilerParams(vmem_limit_bytes=120 * 1024 * 1024),
    )(
        A_x.reshape(S, DM).T, A_c_kv.reshape(S, DC), A_w_q, A_w_uk, A_w_uv,
        jnp.swapaxes(A_w_o, 1, 2),
        B_x.reshape(S, DM).T, B_mem0.reshape(M, DM), B_Wq, B_Wk, B_Wv,
        jnp.swapaxes(B_Wo, 1, 2),
    )
    return out.reshape(1, S, 2 * DM)
```
